```python
import os as _os
_os.environ.setdefault("JAX_PLATFORMS", "cpu")
import jax
import jax.numpy as jnp

def _softmax(x, axis=-1):
    return jax.nn.softmax(x, axis=axis)
def _gelu(x):
    return jax.nn.gelu(x, approximate=True)
def _silu(x):
    return jax.nn.silu(x)
def _sigmoid(x):
    return jax.nn.sigmoid(x)
def _layernorm(x, axis=-1, eps=1e-5):
    m = jnp.mean(x, axis=axis, keepdims=True)
    v = jnp.var(x, axis=axis, keepdims=True)
    return (x - m) / jnp.sqrt(v + eps)
def _scatter_add(tgt, idx, src, axis=0):
    return tgt.at[idx].add(src)
def _segment_sum(src, seg, n):
    return jax.ops.segment_sum(src, seg, n)
class _Rng:
    def __init__(self, key):
        self._k = key
    def _next(self):
        self._k, sub = jax.random.split(self._k)
        return sub
    def normal(self, shape):
        return jax.random.normal(self._next(), shape, dtype=jnp.bfloat16)
    def randint(self, lo, hi, shape):
        return jax.random.randint(self._next(), shape, lo, hi, dtype=jnp.int32)
    def uniform(self, shape, lo=0.0, hi=1.0):
        return jax.random.uniform(self._next(), shape, jnp.bfloat16, lo, hi)
    def permutation(self, n):
        return jax.random.permutation(self._next(), n)


kernel_name = 'concat_heads__mha_block_cached__mha_block_cached__near_ridge'

def setup_inputs():
    _rng = _Rng(jax.random.key(int.from_bytes(__import__("os").urandom(4), "little")))
    _w = (lambda a: (lambda t: t.astype(jnp.bfloat16) if jnp.issubdtype(t.dtype, jnp.floating) else t)(jnp.asarray(a)))
    def _A_setup():
        B, Sq, D = 32, 32, 640
        H, Sk, Dh = 32, 32, 128
        return {
            "x": _w((lambda *s: _rng.normal(s) * 0.8)(B, Sq, D)),
            "k_cache": _w((lambda *s: _rng.normal(s) * 0.8)(B, H, Sk, Dh)),
            "v_cache": _w((lambda *s: _rng.normal(s) * 0.05)(B, H, Sk, Dh)),
            "wq": _w((lambda *s: _rng.normal(s) * 0.8)(D, H * Dh) * (D ** -0.5)),
            "wo": _w((lambda *s: _rng.normal(s) * 0.05)(H * Dh, D) * ((H * Dh) ** -0.5)),
        }
    _A_in = _A_setup()

    def _B_setup():
        B, Sq, D = 32, 32, 640
        H, Sk, Dh = 32, 32, 128
        return {
            "x": _w((lambda *s: _rng.normal(s) * 0.8)(B, Sq, D)),
            "k_cache": _w((lambda *s: _rng.normal(s) * 0.8)(B, H, Sk, Dh)),
            "v_cache": _w((lambda *s: _rng.normal(s) * 0.05)(B, H, Sk, Dh)),
            "wq": _w((lambda *s: _rng.normal(s) * 0.8)(D, H * Dh) * (D ** -0.5)),
            "wo": _w((lambda *s: _rng.normal(s) * 0.05)(H * Dh, D) * ((H * Dh) ** -0.5)),
        }
    _B_in = _B_setup()

    return {
        "A_x": _A_in["x"],
        "A_k_cache": _A_in["k_cache"],
        "A_v_cache": _A_in["v_cache"],
        "A_wq": _A_in["wq"],
        "A_wo": _A_in["wo"],
        "B_x": _B_in["x"],
        "B_k_cache": _B_in["k_cache"],
        "B_v_cache": _B_in["v_cache"],
        "B_wq": _B_in["wq"],
        "B_wo": _B_in["wo"],
    }

def reference(A_x, A_k_cache, A_v_cache, A_wq, A_wo, B_x, B_k_cache, B_v_cache, B_wq, B_wo):
    def _A_ref(x, k_cache, v_cache, wq, wo):
        B, Sq, D = x.shape
        H, Dh = 32, 128
        q = (lambda x, *d: x.transpose(*d))((x @ wq).reshape(B, Sq, H, Dh), 0, 2, 1, 3)
        scores = jnp.einsum("bhqd,bhkd->bhqk", q, k_cache) * (Dh ** -0.5)
        p = _softmax(scores, axis=-1)
        o = jnp.einsum("bhqk,bhkd->bhqd", p, v_cache)
        return (lambda x, *d: x.transpose(*d))(o, 0, 2, 1, 3).reshape(B, Sq, H * Dh) @ wo

    def _B_ref(x, k_cache, v_cache, wq, wo):
        B, Sq, D = x.shape
        H, Dh = 32, 128
        q = (lambda x, *d: x.transpose(*d))((x @ wq).reshape(B, Sq, H, Dh), 0, 2, 1, 3)
        scores = jnp.einsum("bhqd,bhkd->bhqk", q, k_cache) * (Dh ** -0.5)
        p = _softmax(scores, axis=-1)
        o = jnp.einsum("bhqk,bhkd->bhqd", p, v_cache)
        return (lambda x, *d: x.transpose(*d))(o, 0, 2, 1, 3).reshape(B, Sq, H * Dh) @ wo

    a = _A_ref(A_x, A_k_cache, A_v_cache, A_wq, A_wo)
    b = _B_ref(B_x, B_k_cache, B_v_cache, B_wq, B_wo)
    return jnp.concatenate([a, b], axis=-1)
```

```python
import numpy as np

import jax
import jax.numpy as jnp
from jax import lax
import jax.experimental.pallas as pl
import jax.experimental.pallas.tpu as pltpu

F32, BF16 = jnp.float32, jnp.bfloat16

B, SQ, D = 32, 32, 640
H, SK, DH = 32, 32, 128
HD = H * DH
R = B * SQ
QB = 4
G = B // QB
GM = QB * SQ

HG = 4
U = 2
NG = G // U
U0 = 2
U3 = 2
CW = 512

_C = np.float32(DH ** -0.5 * np.log2(np.e))
_NT = (((1,), (1,)), ((), ()))

_RAMP_COPIES = (("w", 0, 512), ("x", 0, 256), ("x", 256, 512), ("x", 512, R),
                ("w", 512, 1024), ("w", 1024, 2048), ("w", 2048, HD))
_RAMP_STEPS = (((0, 1), (0, 256, 0, 512)), ((2,), (256, 512, 0, 512)), ((3,), (512, R, 0, 512)),
               ((4,), (0, R, 512, 1024)), ((5,), (0, R, 1024, 2048)))
_RAMP_LAST_WAIT = 6
_RAMP_COLS = 2048


def _mm(a, b):
    return jnp.dot(a, b, preferred_element_type=F32)


def _softmax_pv(s, v4):
    row = lax.broadcasted_iota(jnp.int32, (GM, GM), 0) >> 5
    col = lax.broadcasted_iota(jnp.int32, (GM, GM), 1) >> 5
    s = jnp.where(row == col, s, -jnp.inf)
    m = jnp.max(s, axis=1, keepdims=True)
    e = jnp.exp2((s - m) * _C)
    l = jnp.sum(e, axis=1, keepdims=True)
    o = _mm(e.astype(BF16), v4)
    r = pl.reciprocal(l, approx=True)
    r = r * (2.0 - l * r)
    return (o * r).astype(BF16)


def _kernel(ax, ak, av, awq, awo, bx, bk, bv, bwq, bwo, out,
            xa_s, xb_s, wqa_s, wqb_s, woa_s, wob_s, ka_s, va_s, kb_s, vb_s,
            qa_s, qb_s, oa_s, ob_s, outa_s, outb_s, acc_s, sems, kv_sems, out_sem):
    ramp = []
    for i, (kind, lo, hi) in enumerate(_RAMP_COPIES):
        if kind == "w":
            ramp.append(pltpu.make_async_copy(
                awq.at[:, pl.ds(lo, hi - lo)], wqa_s.at[:, pl.ds(lo, hi - lo)], sems.at[i]))
        else:
            ramp.append(pltpu.make_async_copy(
                ax.at[pl.ds(lo, hi - lo)], xa_s.at[pl.ds(lo, hi - lo)], sems.at[i]))
    n = len(ramp)
    xb_cp = pltpu.make_async_copy(bx, xb_s, sems.at[n])
    wqb_cp = pltpu.make_async_copy(bwq, wqb_s, sems.at[n + 1])
    woa_cp = pltpu.make_async_copy(awo, woa_s, sems.at[n + 2])
    wob_cp = pltpu.make_async_copy(bwo, wob_s, sems.at[n + 3])

    def kv_copies(br, j):
        pairs = ((ak, ka_s), (av, va_s)) if br == 0 else ((bk, kb_s), (bv, vb_s))
        return [pltpu.make_async_copy(s.at[pl.ds(j * QB * U, QB * U)], d.at[pl.ds(j * QB * U, QB * U)],
                                      kv_sems.at[br * NG + j]) for s, d in pairs]

    def out_copy(br, g):
        src = outa_s if br == 0 else outb_s
        r = g * GM if isinstance(g, int) else pl.multiple_of(g * GM, GM)
        return pltpu.make_async_copy(src.at[pl.ds(r, GM)], out.at[pl.ds(r, GM), pl.ds(br * D, D)], out_sem)

    first = ramp + [xb_cp, wqb_cp]

    def start_first(k, c):
        for kk, cp in enumerate(first):
            @pl.when(k == kk)
            def _():
                cp.start()
        return c

    lax.fori_loop(0, len(first), start_first, 0)

    def start_kv(br):
        def body(j, c):
            for cp in kv_copies(br, j):
                cp.start()
            return c
        lax.fori_loop(0, NG, body, 0)

    start_kv(0)
    woa_cp.start()
    start_kv(1)
    wob_cp.start()

    for waits, (r0, r1, c0, c1) in _RAMP_STEPS:
        for w in waits:
            ramp[w].wait()
        qa_s[r0:r1, c0:c1] = _mm(xa_s[r0:r1, :], wqa_s[:, c0:c1]).astype(BF16)
    ramp[_RAMP_LAST_WAIT].wait()

    def stage0(i, c):
        for u in range(U0):
            cols = pl.ds(pl.multiple_of(_RAMP_COLS + (i * U0 + u) * CW, CW), CW)
            qa_s[:, cols] = _mm(xa_s[...], wqa_s[:, cols]).astype(BF16)
        return c

    lax.fori_loop(0, (HD - _RAMP_COLS) // (CW * U0), stage0, 0)

    NP = H // HG
    PW = HD // NP

    def attn_quad(g, rows, q_s, k_s, v_s, o_s, projection_piece):
        for pc in range(NP):
            heads = range(pc * HG, (pc + 1) * HG)
            scores = []
            for h in heads:
                q = q_s[rows, h * DH:(h + 1) * DH]
                k4 = k_s[pl.ds(g * QB, QB), h].reshape(QB * SK, DH)
                scores.append(lax.dot_general(q, k4, _NT, preferred_element_type=F32))
            projection_piece(pc)
            for h, s in zip(heads, scores):
                v4 = v_s[pl.ds(g * QB, QB), h].reshape(QB * SK, DH)
                o_s[rows, h * DH:(h + 1) * DH] = _softmax_pv(s, v4)

    xb_cp.wait()
    wqb_cp.wait()

    def stage1(i, c):
        for cp in kv_copies(0, i):
            cp.wait()
        for u in range(U):
            g = i * U + u
            rows = pl.ds(pl.multiple_of(g * GM, GM), GM)

            def q_piece(pc, rows=rows):
                cols = slice(pc * PW, (pc + 1) * PW)
                qb_s[rows, cols] = _mm(xb_s[rows, :], wqb_s[:, cols]).astype(BF16)

            attn_quad(g, rows, qa_s, ka_s, va_s, oa_s, q_piece)
        return c

    lax.fori_loop(0, NG, stage1, 0)

    woa_cp.wait()

    def stage2(i, c):
        for cp in kv_copies(1, i):
            cp.wait()
        for u in range(U):
            g = i * U + u
            rows = pl.ds(pl.multiple_of(g * GM, GM), GM)

            def o_piece(pc, rows=rows):
                ks = slice(pc * PW, (pc + 1) * PW)
                part = _mm(oa_s[rows, ks], woa_s[ks, :])
                if pc == 0:
                    acc_s[...] = part
                elif pc < NP - 1:
                    acc_s[...] += part
                else:
                    outa_s[rows, :] = (acc_s[...] + part).astype(BF16)

            attn_quad(g, rows, qb_s, kb_s, vb_s, ob_s, o_piece)
            out_copy(0, g).start()
        return c

    lax.fori_loop(0, NG, stage2, 0)

    wob_cp.wait()

    def stage3(i, c):
        for u in range(U3):
            g = i * U3 + u
            rows = pl.ds(pl.multiple_of(g * GM, GM), GM)
            outb_s[rows, :] = _mm(ob_s[rows, :], wob_s[...]).astype(BF16)
            out_copy(1, g).start()
        return c

    lax.fori_loop(0, G // U3, stage3, 0)

    for br in range(2):
        for g in range(G):
            out_copy(br, g).wait()


@jax.jit
def pallas_concat_heads__mha_block_cached__mha_block_cached__near_ridge_kernel(
    A_x: jax.Array,
    A_k_cache: jax.Array,
    A_v_cache: jax.Array,
    A_wq: jax.Array,
    A_wo: jax.Array,
    B_x: jax.Array,
    B_k_cache: jax.Array,
    B_v_cache: jax.Array,
    B_wq: jax.Array,
    B_wo: jax.Array,
):
    hbm = pl.BlockSpec(memory_space=pl.ANY)
    vmem = pltpu.VMEM
    scratch = (
        [vmem((R, D), BF16)] * 2
        + [vmem((D, HD), BF16)] * 2
        + [vmem((HD, D), BF16)] * 2
        + [vmem((B, H, SK, DH), BF16)] * 4
        + [vmem((R, HD), BF16)] * 4
        + [vmem((R, D), BF16)] * 2
        + [vmem((GM, D), F32)]
        + [pltpu.SemaphoreType.DMA((len(_RAMP_COPIES) + 4,)),
           pltpu.SemaphoreType.DMA((2 * NG,)),
           pltpu.SemaphoreType.DMA(())]
    )
    out = pl.pallas_call(
        _kernel,
        in_specs=[hbm] * 10,
        out_specs=hbm,
        out_shape=jax.ShapeDtypeStruct((R, 2 * D), BF16),
        scratch_shapes=scratch,
        compiler_params=pltpu.CompilerParams(vmem_limit_bytes=110 * 1024 * 1024),
    )(A_x.reshape(R, D), A_k_cache, A_v_cache, A_wq, A_wo,
      B_x.reshape(R, D), B_k_cache, B_v_cache, B_wq, B_wo)
    return out.reshape(B, SQ, 2 * D)
```

```python
import numpy as np

import jax
import jax.numpy as jnp
from jax import lax
import jax.experimental.pallas as pl
import jax.experimental.pallas.tpu as pltpu

F32, BF16 = jnp.float32, jnp.bfloat16

B, SQ, D = 32, 32, 640
H, SK, DH = 32, 32, 128
HD = H * DH
R = B * SQ
QB = 4
G = B // QB
GM = QB * SQ

HG = 4
U = 2
NG = G // U
U0 = 2
U3 = 2
CW = 512

_C = np.float32(DH ** -0.5 * np.log2(np.e))
_NT = (((1,), (1,)), ((), ()))

_RAMP_COPIES = (("w", 0, 512), ("x", 0, 128), ("x", 128, 384), ("x", 384, R),
                ("w", 512, 1024), ("w", 1024, 2048), ("w", 2048, HD))
_RAMP_STEPS = (((0, 1), (0, 128, 0, 512)), ((2,), (128, 384, 0, 512)), ((3,), (384, R, 0, 512)),
               ((4,), (0, R, 512, 1024)), ((5,), (0, R, 1024, 2048)))
_RAMP_LAST_WAIT = 6
_RAMP_COLS = 2048


def _mm(a, b):
    return jnp.dot(a, b, preferred_element_type=F32)


def _softmax_pv(s, v4):
    row = lax.broadcasted_iota(jnp.int32, (GM, GM), 0) >> 5
    col = lax.broadcasted_iota(jnp.int32, (GM, GM), 1) >> 5
    s = jnp.where(row == col, s, -jnp.inf)
    m = jnp.max(s, axis=1, keepdims=True)
    e = jnp.exp2((s - m) * _C)
    l = jnp.sum(e, axis=1, keepdims=True)
    o = _mm(e.astype(BF16), v4)
    return (o * pl.reciprocal(l, approx=True)).astype(BF16)


def _kernel(ax, ak, av, awq, awo, bx, bk, bv, bwq, bwo, out,
            xa_s, xb_s, wqa_s, wqb_s, woa_s, wob_s, ka_s, va_s, kb_s, vb_s,
            qa_s, qb_s, oa_s, ob_s, outa_s, outb_s, acc_s, sems, kv_sems, out_sem):
    ramp = []
    for i, (kind, lo, hi) in enumerate(_RAMP_COPIES):
        if kind == "w":
            ramp.append(pltpu.make_async_copy(
                awq.at[:, pl.ds(lo, hi - lo)], wqa_s.at[:, pl.ds(lo, hi - lo)], sems.at[i]))
        else:
            ramp.append(pltpu.make_async_copy(
                ax.at[pl.ds(lo, hi - lo)], xa_s.at[pl.ds(lo, hi - lo)], sems.at[i]))
    n = len(ramp)
    xb_cp = pltpu.make_async_copy(bx, xb_s, sems.at[n])
    wqb_cp = pltpu.make_async_copy(bwq, wqb_s, sems.at[n + 1])
    woa_cp = pltpu.make_async_copy(awo, woa_s, sems.at[n + 2])
    wob_cp = pltpu.make_async_copy(bwo, wob_s, sems.at[n + 3])

    def kv_copies(br, j):
        pairs = ((ak, ka_s), (av, va_s)) if br == 0 else ((bk, kb_s), (bv, vb_s))
        return [pltpu.make_async_copy(s.at[pl.ds(j * QB * U, QB * U)], d.at[pl.ds(j * QB * U, QB * U)],
                                      kv_sems.at[br * NG + j]) for s, d in pairs]

    def out_copy(br, g, c0, nc):
        src = outa_s if br == 0 else outb_s
        rows = pl.ds(pl.multiple_of(g * GM, GM), GM)
        return pltpu.make_async_copy(src.at[rows, pl.ds(c0, nc)], out.at[rows, pl.ds(br * D + c0, nc)], out_sem)

    first = ramp + [xb_cp, wqb_cp]

    def start_first(k, c):
        for kk, cp in enumerate(first):
            @pl.when(k == kk)
            def _():
                cp.start()
        return c

    lax.fori_loop(0, len(first), start_first, 0)

    def start_kv(br):
        def body(j, c):
            for cp in kv_copies(br, j):
                cp.start()
            return c
        lax.fori_loop(0, NG, body, 0)

    start_kv(0)
    woa_cp.start()
    start_kv(1)
    wob_cp.start()

    for waits, (r0, r1, c0, c1) in _RAMP_STEPS:
        for w in waits:
            ramp[w].wait()
        qa_s[r0:r1, c0:c1] = _mm(xa_s[r0:r1, :], wqa_s[:, c0:c1]).astype(BF16)
    ramp[_RAMP_LAST_WAIT].wait()

    def stage0(i, c):
        for u in range(U0):
            cols = pl.ds(pl.multiple_of(_RAMP_COLS + (i * U0 + u) * CW, CW), CW)
            qa_s[:, cols] = _mm(xa_s[...], wqa_s[:, cols]).astype(BF16)
        return c

    lax.fori_loop(0, (HD - _RAMP_COLS) // (CW * U0), stage0, 0)

    NP = H // HG
    PW = HD // NP

    def attn_quad(g, rows, q_s, k_s, v_s, o_s, projection_piece):
        for pc in range(NP):
            heads = range(pc * HG, (pc + 1) * HG)
            scores = []
            for h in heads:
                q = q_s[rows, h * DH:(h + 1) * DH]
                k4 = k_s[pl.ds(g * QB, QB), h].reshape(QB * SK, DH)
                scores.append(lax.dot_general(q, k4, _NT, preferred_element_type=F32))
            projection_piece(pc)
            for h, s in zip(heads, scores):
                v4 = v_s[pl.ds(g * QB, QB), h].reshape(QB * SK, DH)
                o_s[rows, h * DH:(h + 1) * DH] = _softmax_pv(s, v4)

    xb_cp.wait()
    wqb_cp.wait()

    def stage1(i, c):
        for cp in kv_copies(0, i):
            cp.wait()
        for u in range(U):
            g = i * U + u
            rows = pl.ds(pl.multiple_of(g * GM, GM), GM)

            def q_piece(pc, rows=rows):
                cols = slice(pc * PW, (pc + 1) * PW)
                qb_s[rows, cols] = _mm(xb_s[rows, :], wqb_s[:, cols]).astype(BF16)

            attn_quad(g, rows, qa_s, ka_s, va_s, oa_s, q_piece)
        return c

    lax.fori_loop(0, NG, stage1, 0)

    woa_cp.wait()

    def stage2(i, c):
        for cp in kv_copies(1, i):
            cp.wait()
        for u in range(U):
            g = i * U + u
            rows = pl.ds(pl.multiple_of(g * GM, GM), GM)

            def o_piece(pc, rows=rows):
                ks = slice(pc * PW, (pc + 1) * PW)
                part = _mm(oa_s[rows, ks], woa_s[ks, :])
                if pc == 0:
                    acc_s[...] = part
                elif pc < NP - 1:
                    acc_s[...] += part
                else:
                    outa_s[rows, :] = (acc_s[...] + part).astype(BF16)

            attn_quad(g, rows, qb_s, kb_s, vb_s, ob_s, o_piece)
            out_copy(0, g, 0, D).start()
        return c

    lax.fori_loop(0, NG, stage2, 0)

    wob_cp.wait()

    def stage3(i, c):
        for u in range(U3):
            g = i * U3 + u
            rows = pl.ds(pl.multiple_of(g * GM, GM), GM)
            for c0 in range(0, D, 128):
                outb_s[rows, c0:c0 + 128] = _mm(ob_s[rows, :], wob_s[:, c0:c0 + 128]).astype(BF16)
                out_copy(1, g, c0, 128).start()
        return c

    lax.fori_loop(0, G // U3, stage3, 0)

    pltpu.make_async_copy(out, out, out_sem).wait()


@jax.jit
def pallas_concat_heads__mha_block_cached__mha_block_cached__near_ridge_kernel(
    A_x: jax.Array,
    A_k_cache: jax.Array,
    A_v_cache: jax.Array,
    A_wq: jax.Array,
    A_wo: jax.Array,
    B_x: jax.Array,
    B_k_cache: jax.Array,
    B_v_cache: jax.Array,
    B_wq: jax.Array,
    B_wo: jax.Array,
):
    hbm = pl.BlockSpec(memory_space=pl.ANY)
    vmem = pltpu.VMEM
    scratch = (
        [vmem((R, D), BF16)] * 2
        + [vmem((D, HD), BF16)] * 2
        + [vmem((HD, D), BF16)] * 2
        + [vmem((B, H, SK, DH), BF16)] * 4
        + [vmem((R, HD), BF16)] * 4
        + [vmem((R, D), BF16)] * 2
        + [vmem((GM, D), F32)]
        + [pltpu.SemaphoreType.DMA((len(_RAMP_COPIES) + 4,)),
           pltpu.SemaphoreType.DMA((2 * NG,)),
           pltpu.SemaphoreType.DMA(())]
    )
    out = pl.pallas_call(
        _kernel,
        in_specs=[hbm] * 10,
        out_specs=hbm,
        out_shape=jax.ShapeDtypeStruct((R, 2 * D), BF16),
        scratch_shapes=scratch,
        compiler_params=pltpu.CompilerParams(vmem_limit_bytes=110 * 1024 * 1024),
    )(A_x.reshape(R, D), A_k_cache, A_v_cache, A_wq, A_wo,
      B_x.reshape(R, D), B_k_cache, B_v_cache, B_wq, B_wo)
    return out.reshape(B, SQ, 2 * D)
```

```python
import numpy as np

import jax
import jax.numpy as jnp
from jax import lax
import jax.experimental.pallas as pl
import jax.experimental.pallas.tpu as pltpu

F32, BF16 = jnp.float32, jnp.bfloat16

B, SQ, D = 32, 32, 640
H, SK, DH = 32, 32, 128
HD = H * DH
R = B * SQ
QB = 4
G = B // QB
GM = QB * SQ

HG = 4
U = 2
NG = G // U
U0 = 2
U3 = 2
CW = 512

_C = np.float32(DH ** -0.5 * np.log2(np.e))
_NT = (((1,), (1,)), ((), ()))

_RAMP_COPIES = (("w", 0, 512), ("x", 0, 128), ("x", 128, 384), ("x", 384, R),
                ("w", 512, 1024), ("w", 1024, 2048), ("w", 2048, HD))
_RAMP_STEPS = (((0, 1), (0, 128, 0, 512)), ((2,), (128, 384, 0, 512)), ((3,), (384, R, 0, 512)),
               ((4,), (0, R, 512, 1024)), ((5,), (0, R, 1024, 2048)))
_RAMP_LAST_WAIT = 6
_RAMP_COLS = 2048


def _mm(a, b):
    return jnp.dot(a, b, preferred_element_type=F32)


def _softmax_pv(s, v4):
    row = lax.broadcasted_iota(jnp.int32, (GM, GM), 0) >> 5
    col = lax.broadcasted_iota(jnp.int32, (GM, GM), 1) >> 5
    s = jnp.where(row == col, s, -jnp.inf)
    m = jnp.max(s, axis=1, keepdims=True)
    e = jnp.exp2((s - m) * _C)
    l = jnp.sum(e, axis=1, keepdims=True)
    o = _mm(e.astype(BF16), v4)
    return (o * pl.reciprocal(l, approx=True)).astype(BF16)


def _kernel(ax, ak, av, awq, awo, bx, bk, bv, bwq, bwo, out,
            xa_s, xb_s, wqa_s, wqb_s, woa_s, wob_s, ka_s, va_s, kb_s, vb_s,
            qa_s, qb_s, oa_s, ob_s, outa_s, outb_s, acc_s, sems, kv_sems, out_sem):
    ramp = []
    for i, (kind, lo, hi) in enumerate(_RAMP_COPIES):
        if kind == "w":
            ramp.append(pltpu.make_async_copy(
                awq.at[:, pl.ds(lo, hi - lo)], wqa_s.at[:, pl.ds(lo, hi - lo)], sems.at[i]))
        else:
            ramp.append(pltpu.make_async_copy(
                ax.at[pl.ds(lo, hi - lo)], xa_s.at[pl.ds(lo, hi - lo)], sems.at[i]))
    n = len(ramp)
    xb_cp = pltpu.make_async_copy(bx, xb_s, sems.at[n])
    wqb_cp = pltpu.make_async_copy(bwq, wqb_s, sems.at[n + 1])
    woa_cp = pltpu.make_async_copy(awo, woa_s, sems.at[n + 2])
    wob_cp = pltpu.make_async_copy(bwo, wob_s, sems.at[n + 3])

    def kv_copies(br, j):
        pairs = ((ak, ka_s), (av, va_s)) if br == 0 else ((bk, kb_s), (bv, vb_s))
        return [pltpu.make_async_copy(s.at[pl.ds(j * QB * U, QB * U)], d.at[pl.ds(j * QB * U, QB * U)],
                                      kv_sems.at[br * NG + j]) for s, d in pairs]

    def out_copy(br, g, c0, nc):
        src = outa_s if br == 0 else outb_s
        rows = pl.ds(pl.multiple_of(g * GM, GM), GM)
        return pltpu.make_async_copy(src.at[rows, pl.ds(c0, nc)], out.at[rows, pl.ds(br * D + c0, nc)], out_sem)

    first = ramp + [xb_cp, wqb_cp]

    def start_first(k, c):
        for kk, cp in enumerate(first):
            @pl.when(k == kk)
            def _():
                cp.start()
        return c

    lax.fori_loop(0, len(first), start_first, 0)

    def start_kv(br):
        def body(j, c):
            for cp in kv_copies(br, j):
                cp.start()
            return c
        lax.fori_loop(0, NG, body, 0)

    start_kv(0)
    woa_cp.start()
    start_kv(1)
    wob_cp.start()

    for waits, (r0, r1, c0, c1) in _RAMP_STEPS:
        for w in waits:
            ramp[w].wait()
        qa_s[r0:r1, c0:c1] = _mm(xa_s[r0:r1, :], wqa_s[:, c0:c1]).astype(BF16)
    ramp[_RAMP_LAST_WAIT].wait()

    def stage0(i, c):
        for u in range(U0):
            cols = pl.ds(pl.multiple_of(_RAMP_COLS + (i * U0 + u) * CW, CW), CW)
            qa_s[:, cols] = _mm(xa_s[...], wqa_s[:, cols]).astype(BF16)
        return c

    lax.fori_loop(0, (HD - _RAMP_COLS) // (CW * U0), stage0, 0)

    NP = H // HG
    PW = HD // NP

    def attention_body(i, q_s, k_s, v_s, o_s, projection_piece):
        def rows_of(u):
            return pl.ds(pl.multiple_of((i * U + u) * GM, GM), GM)

        def stacked(ref, u, h):
            return ref[pl.ds((i * U + u) * QB, QB), h].reshape(QB * SK, DH)

        def qk(u, pc):
            return [lax.dot_general(q_s[rows_of(u), h * DH:(h + 1) * DH], stacked(k_s, u, h), _NT,
                                    preferred_element_type=F32)
                    for h in range(pc * HG, (pc + 1) * HG)]

        def softmax_pv(u, pc, scores):
            for h, s in zip(range(pc * HG, (pc + 1) * HG), scores):
                o_s[rows_of(u), h * DH:(h + 1) * DH] = _softmax_pv(s, stacked(v_s, u, h))

        groups = [(u, pc) for u in range(U) for pc in range(NP)]
        pieces = iter(groups)

        def project():
            u, pc = next(pieces)
            projection_piece(u, pc, rows_of(u))

        project()
        s0, s1 = qk(*groups[0]), qk(*groups[1])
        project()
        softmax_pv(*groups[0], s0)
        softmax_pv(*groups[1], s1)
        for grp in groups[2:]:
            s = qk(*grp)
            project()
            softmax_pv(*grp, s)

    xb_cp.wait()
    wqb_cp.wait()

    def stage1(i, c):
        for cp in kv_copies(0, i):
            cp.wait()

        def q_piece(u, pc, rows):
            cols = slice(pc * PW, (pc + 1) * PW)
            qb_s[rows, cols] = _mm(xb_s[rows, :], wqb_s[:, cols]).astype(BF16)

        attention_body(i, qa_s, ka_s, va_s, oa_s, q_piece)
        return c

    lax.fori_loop(0, NG, stage1, 0)

    woa_cp.wait()

    def stage2(i, c):
        for cp in kv_copies(1, i):
            cp.wait()

        def o_piece(u, pc, rows):
            ks = slice(pc * PW, (pc + 1) * PW)
            part = _mm(oa_s[rows, ks], woa_s[ks, :])
            if pc == 0:
                acc_s[...] = part
            elif pc < NP - 1:
                acc_s[...] += part
            else:
                outa_s[rows, :] = (acc_s[...] + part).astype(BF16)
                out_copy(0, i * U + u, 0, D).start()

        attention_body(i, qb_s, kb_s, vb_s, ob_s, o_piece)
        return c

    lax.fori_loop(0, NG, stage2, 0)

    wob_cp.wait()

    def stage3(i, c):
        for u in range(U3):
            g = i * U3 + u
            rows = pl.ds(pl.multiple_of(g * GM, GM), GM)
            for c0 in range(0, D, 128):
                outb_s[rows, c0:c0 + 128] = _mm(ob_s[rows, :], wob_s[:, c0:c0 + 128]).astype(BF16)
                out_copy(1, g, c0, 128).start()
        return c

    lax.fori_loop(0, G // U3, stage3, 0)

    pltpu.make_async_copy(out, out, out_sem).wait()


@jax.jit
def pallas_concat_heads__mha_block_cached__mha_block_cached__near_ridge_kernel(
    A_x: jax.Array,
    A_k_cache: jax.Array,
    A_v_cache: jax.Array,
    A_wq: jax.Array,
    A_wo: jax.Array,
    B_x: jax.Array,
    B_k_cache: jax.Array,
    B_v_cache: jax.Array,
    B_wq: jax.Array,
    B_wo: jax.Array,
):
    hbm = pl.BlockSpec(memory_space=pl.ANY)
    vmem = pltpu.VMEM
    scratch = (
        [vmem((R, D), BF16)] * 2
        + [vmem((D, HD), BF16)] * 2
        + [vmem((HD, D), BF16)] * 2
        + [vmem((B, H, SK, DH), BF16)] * 4
        + [vmem((R, HD), BF16)] * 4
        + [vmem((R, D), BF16)] * 2
        + [vmem((GM, D), F32)]
        + [pltpu.SemaphoreType.DMA((len(_RAMP_COPIES) + 4,)),
           pltpu.SemaphoreType.DMA((2 * NG,)),
           pltpu.SemaphoreType.DMA(())]
    )
    out = pl.pallas_call(
        _kernel,
        in_specs=[hbm] * 10,
        out_specs=hbm,
        out_shape=jax.ShapeDtypeStruct((R, 2 * D), BF16),
        scratch_shapes=scratch,
        compiler_params=pltpu.CompilerParams(vmem_limit_bytes=110 * 1024 * 1024),
    )(A_x.reshape(R, D), A_k_cache, A_v_cache, A_wq, A_wo,
      B_x.reshape(R, D), B_k_cache, B_v_cache, B_wq, B_wo)
    return out.reshape(B, SQ, 2 * D)
```
